```python
import os as _os
_os.environ.setdefault("JAX_PLATFORMS", "cpu")
import jax
import jax.numpy as jnp

def _softmax(x, axis=-1):
    return jax.nn.softmax(x, axis=axis)
def _gelu(x):
    return jax.nn.gelu(x, approximate=True)
def _silu(x):
    return jax.nn.silu(x)
def _sigmoid(x):
    return jax.nn.sigmoid(x)
def _layernorm(x, axis=-1, eps=1e-5):
    m = jnp.mean(x, axis=axis, keepdims=True)
    v = jnp.var(x, axis=axis, keepdims=True)
    return (x - m) / jnp.sqrt(v + eps)
def _scatter_add(tgt, idx, src, axis=0):
    return tgt.at[idx].add(src)
def _segment_sum(src, seg, n):
    return jax.ops.segment_sum(src, seg, n)
class _Rng:
    def __init__(self, key):
        self._k = key
    def _next(self):
        self._k, sub = jax.random.split(self._k)
        return sub
    def normal(self, shape):
        return jax.random.normal(self._next(), shape, dtype=jnp.bfloat16)
    def randint(self, lo, hi, shape):
        return jax.random.randint(self._next(), shape, lo, hi, dtype=jnp.int32)
    def uniform(self, shape, lo=0.0, hi=1.0):
        return jax.random.uniform(self._next(), shape, jnp.bfloat16, lo, hi)
    def permutation(self, n):
        return jax.random.permutation(self._next(), n)


kernel_name = 'concat_heads__sliding_block_cached__sliding_block_cached__decode'

def setup_inputs():
    _rng = _Rng(jax.random.key(int.from_bytes(__import__("os").urandom(4), "little")))
    _w = (lambda a: (lambda t: t.astype(jnp.bfloat16) if jnp.issubdtype(t.dtype, jnp.floating) else t)(jnp.asarray(a)))
    def _A_setup():
        B, Sq, D = 4, 1, 576
        Hq, Hkv, Sk, Dh = 32, 16, 8192, 128
        assert Hq % Hkv == 0, (Hq, Hkv)
        return {
            "x": _w((lambda *s: _rng.normal(s) * 0.8)(B, Sq, D)),
            "k_cache": _w((lambda *s: _rng.normal(s) * 0.8)(B, Hkv, Sk, Dh)),
            "v_cache": _w((lambda *s: _rng.normal(s) * 0.05)(B, Hkv, Sk, Dh)),
            "wq": _w((lambda *s: _rng.normal(s) * 0.8)(D, Hq * Dh) * (D ** -0.5)),
            "wo": _w((lambda *s: _rng.normal(s) * 0.05)(Hq * Dh, D) * ((Hq * Dh) ** -0.5)),
        }
    _A_in = _A_setup()

    def _B_setup():
        B, Sq, D = 4, 1, 576
        Hq, Hkv, Sk, Dh = 32, 16, 8192, 128
        assert Hq % Hkv == 0, (Hq, Hkv)
        return {
            "x": _w((lambda *s: _rng.normal(s) * 0.8)(B, Sq, D)),
            "k_cache": _w((lambda *s: _rng.normal(s) * 0.8)(B, Hkv, Sk, Dh)),
            "v_cache": _w((lambda *s: _rng.normal(s) * 0.05)(B, Hkv, Sk, Dh)),
            "wq": _w((lambda *s: _rng.normal(s) * 0.8)(D, Hq * Dh) * (D ** -0.5)),
            "wo": _w((lambda *s: _rng.normal(s) * 0.05)(Hq * Dh, D) * ((Hq * Dh) ** -0.5)),
        }
    _B_in = _B_setup()

    return {
        "A_x": _A_in["x"],
        "A_k_cache": _A_in["k_cache"],
        "A_v_cache": _A_in["v_cache"],
        "A_wq": _A_in["wq"],
        "A_wo": _A_in["wo"],
        "B_x": _B_in["x"],
        "B_k_cache": _B_in["k_cache"],
        "B_v_cache": _B_in["v_cache"],
        "B_wq": _B_in["wq"],
        "B_wo": _B_in["wo"],
    }

def reference(A_x, A_k_cache, A_v_cache, A_wq, A_wo, B_x, B_k_cache, B_v_cache, B_wq, B_wo):
    def _A_ref(x, k_cache, v_cache, wq, wo):
        B, Sq, D = x.shape
        Hq, Dh = 32, 128
        Hkv, Sk = k_cache.shape[1], k_cache.shape[2]
        W = min(4096, max(256, Sk // 4))
        rep = Hq // Hkv
        q = (lambda x, *d: x.transpose(*d))((x @ wq).reshape(B, Sq, Hq, Dh), 0, 2, 1, 3)
        k = jnp.repeat(k_cache[:, :, Sk - W:, :], rep, axis=1)
        v = jnp.repeat(v_cache[:, :, Sk - W:, :], rep, axis=1)
        scores = jnp.einsum("bhqd,bhkd->bhqk", q, k) * (Dh ** -0.5)
        p = _softmax(scores, axis=-1)
        o = jnp.einsum("bhqk,bhkd->bhqd", p, v)
        return (lambda x, *d: x.transpose(*d))(o, 0, 2, 1, 3).reshape(B, Sq, Hq * Dh) @ wo

    def _B_ref(x, k_cache, v_cache, wq, wo):
        B, Sq, D = x.shape
        Hq, Dh = 32, 128
        Hkv, Sk = k_cache.shape[1], k_cache.shape[2]
        W = min(4096, max(256, Sk // 4))
        rep = Hq // Hkv
        q = (lambda x, *d: x.transpose(*d))((x @ wq).reshape(B, Sq, Hq, Dh), 0, 2, 1, 3)
        k = jnp.repeat(k_cache[:, :, Sk - W:, :], rep, axis=1)
        v = jnp.repeat(v_cache[:, :, Sk - W:, :], rep, axis=1)
        scores = jnp.einsum("bhqd,bhkd->bhqk", q, k) * (Dh ** -0.5)
        p = _softmax(scores, axis=-1)
        o = jnp.einsum("bhqk,bhkd->bhqd", p, v)
        return (lambda x, *d: x.transpose(*d))(o, 0, 2, 1, 3).reshape(B, Sq, Hq * Dh) @ wo

    a = _A_ref(A_x, A_k_cache, A_v_cache, A_wq, A_wo)
    b = _B_ref(B_x, B_k_cache, B_v_cache, B_wq, B_wo)
    return jnp.concatenate([a, b], axis=-1)
```

```python
import functools

import jax
import jax.numpy as jnp
from jax import lax
import jax.experimental.pallas as pl
import jax.experimental.pallas.tpu as pltpu

_NT = (((1,), (1,)), ((), ()))


def build(depth=3, prio=True, do_compute=True):
    def entry(A_x, A_k, A_v, A_wq, A_wo, B_x, B_k, B_v, B_wq, B_wo):
        B, Sq, D = A_x.shape
        Hq, Dh = 32, 128
        Hkv, Sk = A_k.shape[1], A_k.shape[2]
        W = min(4096, max(256, Sk // 4))
        rep = Hq // Hkv
        assert Sq == 1 and B * rep == 8 and rep == 2
        scale = Dh ** -0.5
        NS = 2 * Hkv
        f32, bf16 = jnp.float32, jnp.bfloat16

        def kernel(xa, ka, va, wqa, woa, xb, kb, vb, wqb, wob, out_ref,
                   xbuf, wqbuf, wobuf, kbuf, vbuf, q_scr, o_scr, res_scr,
                   xsem, wqsem, wosem, ksem, vsem):
            def kv_copies(k_ref, v_ref, h, slot):
                return (
                    pltpu.make_async_copy(k_ref.at[:, h, pl.ds(Sk - W, W), :], kbuf.at[slot], ksem.at[slot]),
                    pltpu.make_async_copy(v_ref.at[:, h, pl.ds(Sk - W, W), :], vbuf.at[slot], vsem.at[slot]),
                )

            def start_kv(k_ref, v_ref, h, slot):
                ck, cv = kv_copies(k_ref, v_ref, h, slot)
                ck.start()
                cv.start(priority=1 if prio else 0)

            x_cp = [pltpu.make_async_copy(r, xbuf.at[i], xsem.at[i]) for i, r in enumerate((xa, xb))]
            wq_cp = [pltpu.make_async_copy(r, wqbuf.at[i], wqsem.at[i]) for i, r in enumerate((wqa, wqb))]
            wo_cp = [pltpu.make_async_copy(r, wobuf.at[i], wosem.at[i]) for i, r in enumerate((woa, wob))]

            wq_cp[0].start()
            x_cp[0].start()
            x_cp[1].start()
            for s in range(depth):
                start_kv(ka, va, s, s)

            row = lax.broadcasted_iota(jnp.int32, (8, Dh), 0)

            def q_proj(i):
                x_cp[i].wait()
                wq_cp[i].wait()
                if not do_compute:
                    return
                x4 = xbuf[i].astype(f32)
                x8 = jnp.concatenate([x4, x4], axis=0).astype(bf16)
                for h in range(Hkv):
                    q = jnp.dot(x8, wqbuf[i, :, h * 256:(h + 1) * 256], preferred_element_type=f32)
                    q_scr[i * Hkv + h] = jnp.where(row < B, q[:, :Dh], q[:, Dh:])

            def out_proj(i):
                wo_cp[i].wait()
                if not do_compute:
                    return jnp.zeros((8, D), f32)
                o = jnp.concatenate([o_scr[i * Hq + j] for j in range(Hq)], axis=1).astype(bf16)
                return lax.dot_general(o, wobuf[i], _NT, preferred_element_type=f32)

            def attend(s, slot):
                ck, cv = kv_copies(ka, va, 0, slot)
                ck.wait()
                if do_compute:
                    q = q_scr[s].astype(bf16)
                    rowb = lax.broadcasted_iota(jnp.int32, (8, W), 0) % B
                    sc = None
                    for b in range(B):
                        sb = lax.dot_general(q, kbuf[slot, b], _NT, preferred_element_type=f32)
                        sc = sb if b == 0 else jnp.where(rowb == b, sb, sc)
                    sc = sc * scale
                    m = jnp.max(sc, axis=1, keepdims=True)
                    e = jnp.exp(sc - m)
                    l = jnp.sum(e, axis=1, keepdims=True)
                    p = e.astype(bf16)
                cv.wait()
                if do_compute:
                    o = None
                    for b in range(B):
                        ob = jnp.dot(p, vbuf[slot, b], preferred_element_type=f32)
                        o = ob if b == 0 else jnp.where(row % B == b, ob, o)
                    o = o / l
                    o_scr[2 * s] = o
                    o_scr[2 * s + 1] = pltpu.roll(o, B, 0)

            q_proj(0)

            def body(s, _):
                slot = lax.rem(s, depth)

                @pl.when(s == 4)
                def _():
                    wq_cp[1].start()

                @pl.when(s == 8)
                def _():
                    q_proj(1)

                @pl.when(s == Hkv)
                def _():
                    wo_cp[0].start()

                @pl.when(s == Hkv + 4)
                def _():
                    res_scr[...] = out_proj(0)

                attend(s, slot)
                n = s + depth

                @pl.when(n < Hkv)
                def _():
                    start_kv(ka, va, n, slot)

                @pl.when(jnp.logical_and(n >= Hkv, n < NS))
                def _():
                    start_kv(kb, vb, n - Hkv, slot)

                @pl.when(n == NS)
                def _():
                    wo_cp[1].start()

            lax.fori_loop(0, NS, body, None)
            rb = out_proj(1)
            out_ref[...] = jnp.concatenate([res_scr[0:B, :], rb[0:B, :]], axis=1).astype(out_ref.dtype)

        any_spec = pl.BlockSpec(memory_space=pl.ANY)
        out = pl.pallas_call(
            kernel,
            out_shape=jax.ShapeDtypeStruct((B, 2 * D), A_x.dtype),
            in_specs=[any_spec] * 10,
            out_specs=pl.BlockSpec(memory_space=pltpu.VMEM),
            scratch_shapes=[
                pltpu.VMEM((2, B, D), bf16),
                pltpu.VMEM((2, D, Hq * Dh), bf16),
                pltpu.VMEM((2, D, Hq * Dh), bf16),
                pltpu.VMEM((depth, B, W, Dh), bf16),
                pltpu.VMEM((depth, B, W, Dh), bf16),
                pltpu.VMEM((NS, 8, Dh), f32),
                pltpu.VMEM((2 * NS, 8, Dh), f32),
                pltpu.VMEM((8, D), f32),
                pltpu.SemaphoreType.DMA((2,)),
                pltpu.SemaphoreType.DMA((2,)),
                pltpu.SemaphoreType.DMA((2,)),
                pltpu.SemaphoreType.DMA((depth,)),
                pltpu.SemaphoreType.DMA((depth,)),
            ],
            compiler_params=pltpu.CompilerParams(vmem_limit_bytes=100 * 2**20),
        )(A_x.reshape(B, D), A_k, A_v, A_wq, A_wo.T, B_x.reshape(B, D), B_k, B_v, B_wq, B_wo.T)
        return out.reshape(B, Sq, 2 * D)

    return entry


@jax.jit
def pallas_concat_heads__sliding_block_cached__sliding_block_cached__decode_kernel(A_x, A_k_cache, A_v_cache, A_wq, A_wo, B_x, B_k_cache, B_v_cache, B_wq, B_wo):
    return build(depth=3,prio=False)(A_x, A_k_cache, A_v_cache, A_wq, A_wo, B_x, B_k_cache, B_v_cache, B_wq, B_wo)
```

```python
import functools

import jax
import jax.numpy as jnp
from jax import lax
import jax.experimental.pallas as pl
import jax.experimental.pallas.tpu as pltpu

_NT = (((1,), (1,)), ((), ()))


def build(ahead=20, rows=512, r0=192, w0=112, do_compute=True, nobounds=True, order="bc"):
    def entry(A_x, A_k, A_v, A_wq, A_wo, B_x, B_k, B_v, B_wq, B_wo):
        B, Sq, D = A_x.shape
        Hq, Dh = 32, 128
        Hkv, Sk = A_k.shape[1], A_k.shape[2]
        W = min(4096, max(256, Sk // 4))
        rep = Hq // Hkv
        assert Sq == 1 and B * rep == 8 and rep == 2
        scale = Dh ** -0.5
        NS = 2 * Hkv
        G = rep * Dh
        NC = W // rows
        f32, bf16 = jnp.float32, jnp.bfloat16

        if order == "bc":
            bc = [(b, c) for b in range(B) for c in range(NC)]
        else:
            bc = [(b, c) for c in range(NC) for b in range(B)]
        units = ([("wq", j, 0) for j in range(2)] + [("k", b, c) for b, c in bc]
                 + [("v", b, c) for b, c in bc] + [("wo", j, 0) for j in range(2)])
        NU = len(units)
        assert ahead <= NU - 2

        def kernel(xa, ka, va, wqa, woa, xb, kb, vb, wqb, wob, out_ref,
                   xbuf, x_scr, wqbuf, wobuf, kbuf, vbuf, acc, xsem, sems):
            hbm = (dict(k=ka, v=va, wq=wqa, wo=woa), dict(k=kb, v=vb, wq=wqb, wo=wob))
            vmem = dict(k=kbuf, v=vbuf, wq=wqbuf, wo=wobuf)

            def copies(i, h, u):
                kind, a, c = units[u]
                src, dst = hbm[i][kind], vmem[kind]
                if kind in ("k", "v"):
                    parts = ((c * rows, r0), (c * rows + r0, rows - r0))
                    return [pltpu.make_async_copy(src.at[a, h, pl.ds(Sk - W + o, n), :],
                                                  dst.at[a, pl.ds(o, n), :], sems.at[u])
                            for o, n in parts]
                half = D // 2
                parts = ((a * half, w0), (a * half + w0, half - w0))
                col = h * G if isinstance(h, int) else pl.multiple_of(h * G, G)
                return [pltpu.make_async_copy(src.at[pl.ds(o, n), pl.ds(col, G)],
                                              dst.at[pl.ds(o, n), :], sems.at[u])
                        for o, n in parts]

            def start(i, h, u):
                for prio, cp in enumerate(copies(i, h, u)):
                    cp.start(priority=prio)

            def wait(u):
                for cp in copies(0, 0, u):
                    cp.wait()

            x_cp = [pltpu.make_async_copy(r, xbuf.at[i], xsem.at[i]) for i, r in enumerate((xa, xb))]
            start(0, 0, 0)
            x_cp[0].start()
            x_cp[1].start()
            for u in range(1, ahead):
                start(0, 0, u)

            acc[...] = jnp.zeros_like(acc)
            for i in range(2):
                x_cp[i].wait()
                x4 = xbuf[i].astype(f32)
                x_scr[i] = jnp.concatenate([x4, x4], axis=0)

            row = lax.broadcasted_iota(jnp.int32, (8, Dh), 0)
            rowb = lax.broadcasted_iota(jnp.int32, (8, rows), 0) % B

            def body(s, _):
                br = s // Hkv

                def advance(u):
                    wait(u)
                    n, un = (s, u + ahead) if u + ahead < NU else (s + 1, u + ahead - NU)

                    @pl.when(n < Hkv)
                    def _():
                        start(0, n, un)

                    @pl.when(jnp.logical_and(n >= Hkv, n < NS))
                    def _():
                        start(1, n - Hkv, un)

                if not do_compute:
                    for u in range(NU):
                        advance(u)
                    return

                advance(0)
                advance(1)
                q = jnp.dot(x_scr[br].astype(bf16), wqbuf[...], preferred_element_type=f32)
                q = jnp.where(row < B, q[:, :Dh], q[:, Dh:]).astype(bf16)
                u = 2
                sc = [None] * NC
                for b, c in bc:
                    advance(u)
                    u += 1
                    sb = lax.dot_general(q, kbuf[b, c * rows:(c + 1) * rows, :], _NT,
                                         preferred_element_type=f32)
                    sc[c] = sb if b == 0 else jnp.where(rowb == b, sb, sc[c])
                sc = [t * scale for t in sc]
                m = jnp.max(functools.reduce(jnp.maximum, sc), axis=1, keepdims=True)
                e = [jnp.exp(t - m) for t in sc]
                l = jnp.sum(functools.reduce(jnp.add, e), axis=1, keepdims=True)
                p = [t.astype(bf16) for t in e]
                ob = [None] * B
                for b, c in bc:
                    advance(u)
                    u += 1
                    t = jnp.dot(p[c], vbuf[b, c * rows:(c + 1) * rows, :], preferred_element_type=f32)
                    ob[b] = t if c == 0 else ob[b] + t
                o = ob[0]
                for b in range(1, B):
                    o = jnp.where(row % B == b, ob[b], o)
                o = o / l
                lhs = jnp.concatenate([o, pltpu.roll(o, B, 0)], axis=1).astype(bf16)
                advance(u)
                advance(u + 1)
                acc[br] += lax.dot_general(lhs, wobuf[...], _NT, preferred_element_type=f32)

            lax.fori_loop(0, NS, body, None)
            out_ref[...] = jnp.concatenate([acc[0, 0:B, :], acc[1, 0:B, :]], axis=1).astype(out_ref.dtype)

        any_spec = pl.BlockSpec(memory_space=pl.ANY)
        out = pl.pallas_call(
            kernel,
            out_shape=jax.ShapeDtypeStruct((B, 2 * D), A_x.dtype),
            in_specs=[any_spec] * 10,
            out_specs=pl.BlockSpec(memory_space=pltpu.VMEM),
            scratch_shapes=[
                pltpu.VMEM((2, B, D), bf16),
                pltpu.VMEM((2, 8, D), f32),
                pltpu.VMEM((D, G), bf16),
                pltpu.VMEM((D, G), bf16),
                pltpu.VMEM((B, W, Dh), bf16),
                pltpu.VMEM((B, W, Dh), bf16),
                pltpu.VMEM((2, 8, D), f32),
                pltpu.SemaphoreType.DMA((2,)),
                pltpu.SemaphoreType.DMA((NU,)),
            ],
            compiler_params=pltpu.CompilerParams(disable_bounds_checks=nobounds),
        )(A_x.reshape(B, D), A_k, A_v, A_wq, A_wo.T, B_x.reshape(B, D), B_k, B_v, B_wq, B_wo.T)
        return out.reshape(B, Sq, 2 * D)

    return entry


@jax.jit
def pallas_concat_heads__sliding_block_cached__sliding_block_cached__decode_kernel(A_x, A_k_cache, A_v_cache, A_wq, A_wo, B_x, B_k_cache, B_v_cache, B_wq, B_wo):
    return build(order='cb')(A_x, A_k_cache, A_v_cache, A_wq, A_wo, B_x, B_k_cache, B_v_cache, B_wq, B_wo)
```

```python
import functools

import jax
import jax.numpy as jnp
from jax import lax
import jax.experimental.pallas as pl
import jax.experimental.pallas.tpu as pltpu

_HQ, _DH = 32, 128
_NT = (((1,), (1,)), ((), ()))

_CHUNK = 512
_CHUNK_UNITS = (((0, 192, 1), (192, 16, 0)), ((208, 240, 1), (448, 64, 0)))
_WEIGHT_UNITS = tuple(((r, 64, 0), (r + 64, 128, 1)) for r in (0, 192, 384))
_AHEAD = 46


def _extent(pieces):
    return pieces[0][0], sum(n for _, n, _ in pieces)


@jax.jit
def pallas_concat_heads__sliding_block_cached__sliding_block_cached__decode_kernel(
    A_x: jax.Array,
    A_k_cache: jax.Array,
    A_v_cache: jax.Array,
    A_wq: jax.Array,
    A_wo: jax.Array,
    B_x: jax.Array,
    B_k_cache: jax.Array,
    B_v_cache: jax.Array,
    B_wq: jax.Array,
    B_wo: jax.Array,
):
    B, Sq, D = A_x.shape
    Hkv, Sk = A_k_cache.shape[1], A_k_cache.shape[2]
    W = min(4096, max(256, Sk // 4))
    rep = _HQ // Hkv
    group = rep * _DH
    n_steps = 2 * Hkv
    n_chunks = W // _CHUNK
    pad = -D % 128
    Dp = D + pad
    dtype = A_x.dtype
    f32 = jnp.float32
    assert A_x.shape == B_x.shape and A_k_cache.shape == B_k_cache.shape
    assert Sq == 1 and rep == 2 and rep * B == 8 and W % _CHUNK == 0
    assert sum(_extent(_WEIGHT_UNITS[-1])) == D and 2 * pad == 128

    def cache_units(kind):
        return [(kind, b, c, pieces)
                for c in range(n_chunks) for pieces in _CHUNK_UNITS for b in range(B)]

    def weight_units(kind):
        return [(kind, 0, 0, pieces) for pieces in _WEIGHT_UNITS]

    units = weight_units("wq") + cache_units("k") + cache_units("v") + weight_units("wo")
    n_units = len(units)
    assert _AHEAD < n_units - B

    def kernel(xa, ka, va, wqa, woa, xb, kb, vb, wqb, wob, out_ref,
               x_buf, x_rows, wq_buf, wo_buf, k_buf, v_buf, out_a, x_sems, sems):
        hbm = (dict(k=ka, v=va, wq=wqa, wo=woa), dict(k=kb, v=vb, wq=wqb, wo=wob))
        vmem = dict(k=k_buf, v=v_buf, wq=wq_buf, wo=wo_buf)

        def scaled(i, n):
            return i * n if isinstance(i, int) else pl.multiple_of(i * n, n)

        def landing(branch, u, first, n):
            kind, b, c, _ = units[u]
            if kind in ("k", "v"):
                return vmem[kind].at[b, pl.ds(c * _CHUNK + first, n), :]
            if kind == "wo":
                first = scaled(first // pad + branch, pad)
            return vmem[kind].at[pl.ds(first, n), :]

        def start(branch, head, u):
            kind, b, c, pieces = units[u]
            for first, n, priority in sorted(pieces, key=lambda piece: piece[2]):
                if kind in ("k", "v"):
                    src = hbm[branch][kind].at[b, head, pl.ds(Sk - W + c * _CHUNK + first, n), :]
                else:
                    src = hbm[branch][kind].at[pl.ds(first, n), pl.ds(scaled(head, group), group)]
                pltpu.make_async_copy(
                    src, landing(branch, u, first, n), sems.at[u]).start(priority=priority)

        def wait(branch, u):
            filled = landing(branch, u, *_extent(units[u][3]))
            pltpu.make_async_copy(filled, filled, sems.at[u]).wait()

        wo_buf[D:, :] = jnp.zeros((pad, group), dtype)
        x_copies = [pltpu.make_async_copy(x, x_buf.at[i], x_sems.at[i])
                    for i, x in enumerate((xa, xb))]
        for copy in x_copies:
            copy.start()
        for u in range(_AHEAD):
            start(0, 0, u)
        for i, copy in enumerate(x_copies):
            copy.wait()
            x = x_buf[i].astype(f32)
            x_rows[i] = jnp.concatenate([x, x], axis=0)

        row = lax.broadcasted_iota(jnp.int32, (8, _DH), 0)
        score_batch = lax.broadcasted_iota(jnp.int32, (8, _CHUNK), 0) % B

        def step(s, acc):
            branch = s // Hkv

            @pl.when(s == Hkv)
            def _():
                out_a[...] = acc

            acc = jnp.where(s == Hkv, 0.0, acc)

            def advance(u):
                wait(branch, u)
                wraps, v = divmod(u + _AHEAD, n_units)
                t = s + wraps

                @pl.when(t < Hkv)
                def _():
                    start(0, t, v)

                @pl.when(jnp.logical_and(t >= Hkv, t < n_steps))
                def _():
                    start(1, t - Hkv, v)

            q = probs = denom = heads = None
            scores = [None] * n_chunks
            pv = [None] * B
            new_acc, done = [], 0
            for u, (kind, b, c, pieces) in enumerate(units):
                advance(u)
                landed = sum(_extent(pieces))
                rows = pl.ds(c * _CHUNK, _CHUNK)
                final = (b, c) == (B - 1, n_chunks - 1)
                if kind == "wq" and landed == D:
                    q = jnp.dot(x_rows[branch].astype(dtype), wq_buf[...],
                                preferred_element_type=f32)
                    q = jnp.where(row < B, q[:, :_DH], q[:, _DH:]).astype(dtype)
                elif kind == "k" and landed == _CHUNK:
                    part = lax.dot_general(q, k_buf[b, rows, :], _NT, preferred_element_type=f32)
                    scores[c] = part if b == 0 else jnp.where(score_batch == b, part, scores[c])
                    if final:
                        scores = [x * _DH ** -0.5 for x in scores]
                        top = jnp.max(functools.reduce(jnp.maximum, scores), axis=1, keepdims=True)
                        exps = [jnp.exp(x - top) for x in scores]
                        denom = jnp.sum(functools.reduce(jnp.add, exps), axis=1, keepdims=True)
                        probs = [x.astype(dtype) for x in exps]
                elif kind == "v" and landed == _CHUNK:
                    part = jnp.dot(probs[c], v_buf[b, rows, :], preferred_element_type=f32)
                    pv[b] = part if c == 0 else pv[b] + part
                    if final:
                        o = pv[0]
                        for other in range(1, B):
                            o = jnp.where(row % B == other, pv[other], o)
                        o = o / denom
                        heads = jnp.concatenate([o, pltpu.roll(o, B, 0)], axis=1).astype(dtype)
                elif kind == "wo":
                    ready = Dp if landed == D else landed // 128 * 128
                    new_acc.append(acc[:, done:ready] + lax.dot_general(
                        heads, wo_buf[done:ready, :], _NT, preferred_element_type=f32))
                    done = ready
            return jnp.concatenate(new_acc, axis=1)

        out_b = lax.fori_loop(0, n_steps, step, jnp.zeros((8, Dp), f32))

        lane = lax.broadcasted_iota(jnp.int32, (8, 128), 1)
        seam = jnp.where(lane < 128 - pad, out_a[:, Dp - 128:], out_b[:, :128])
        out = jnp.concatenate([out_a[:, :Dp - 128], seam, out_b[:, 128:]], axis=1)
        out_ref[...] = out[:B].astype(dtype)

    out = pl.pallas_call(
        kernel,
        out_shape=jax.ShapeDtypeStruct((B, 2 * D), dtype),
        in_specs=[pl.BlockSpec(memory_space=pl.ANY)] * 10,
        out_specs=pl.BlockSpec(memory_space=pltpu.VMEM),
        scratch_shapes=[
            pltpu.VMEM((2, B, D), dtype),
            pltpu.VMEM((2, 8, D), f32),
            pltpu.VMEM((D, group), dtype),
            pltpu.VMEM((Dp, group), dtype),
            pltpu.VMEM((B, W, _DH), dtype),
            pltpu.VMEM((B, W, _DH), dtype),
            pltpu.VMEM((8, Dp), f32),
            pltpu.SemaphoreType.DMA((2,)),
            pltpu.SemaphoreType.DMA((n_units,)),
        ],
        compiler_params=pltpu.CompilerParams(
            disable_bounds_checks=True, disable_semaphore_checks=True),
    )(A_x.reshape(B, D), A_k_cache, A_v_cache, A_wq, A_wo.T,
      B_x.reshape(B, D), B_k_cache, B_v_cache, B_wq, B_wo.T)
    return out.reshape(B, Sq, 2 * D)
```
